```python
import os as _os
_os.environ.setdefault("JAX_PLATFORMS", "cpu")
import jax
import jax.numpy as jnp

def _softmax(x, axis=-1):
    return jax.nn.softmax(x, axis=axis)
def _gelu(x):
    return jax.nn.gelu(x, approximate=True)
def _silu(x):
    return jax.nn.silu(x)
def _sigmoid(x):
    return jax.nn.sigmoid(x)
def _layernorm(x, axis=-1, eps=1e-5):
    m = jnp.mean(x, axis=axis, keepdims=True)
    v = jnp.var(x, axis=axis, keepdims=True)
    return (x - m) / jnp.sqrt(v + eps)
def _scatter_add(tgt, idx, src, axis=0):
    return tgt.at[idx].add(src)
def _segment_sum(src, seg, n):
    return jax.ops.segment_sum(src, seg, n)
class _Rng:
    def __init__(self, key):
        self._k = key
    def _next(self):
        self._k, sub = jax.random.split(self._k)
        return sub
    def normal(self, shape):
        return jax.random.normal(self._next(), shape, dtype=jnp.bfloat16)
    def randint(self, lo, hi, shape):
        return jax.random.randint(self._next(), shape, lo, hi, dtype=jnp.int32)
    def uniform(self, shape, lo=0.0, hi=1.0):
        return jax.random.uniform(self._next(), shape, jnp.bfloat16, lo, hi)
    def permutation(self, n):
        return jax.random.permutation(self._next(), n)


kernel_name = 'standalone__gqa_block_cached__sampling'

def setup_inputs():
    _rng = _Rng(jax.random.key(int.from_bytes(__import__("os").urandom(4), "little")))
    _w = (lambda a: (lambda t: t.astype(jnp.bfloat16) if jnp.issubdtype(t.dtype, jnp.floating) else t)(jnp.asarray(a)))
    B, Sq, D = 32, 16, 1024
    Hq, Hkv, Sk, Dh = 32, 4, 2048, 128
    assert Hq % Hkv == 0, (Hq, Hkv)
    return {
        "x": _w((lambda *s: _rng.normal(s) * 0.8)(B, Sq, D)),
        "k_cache": _w((lambda *s: _rng.normal(s) * 0.8)(B, Hkv, Sk, Dh)),
        "v_cache": _w((lambda *s: _rng.normal(s) * 0.05)(B, Hkv, Sk, Dh)),
        "wq": _w((lambda *s: _rng.normal(s) * 0.8)(D, Hq * Dh) * (D ** -0.5)),
        "wo": _w((lambda *s: _rng.normal(s) * 0.05)(Hq * Dh, D) * ((Hq * Dh) ** -0.5)),
    }

def reference(x, k_cache, v_cache, wq, wo):
    B, Sq, D = x.shape
    Hq, Dh = 32, 128
    Hkv = k_cache.shape[1]
    rep = Hq // Hkv
    q = (lambda x, *d: x.transpose(*d))((x @ wq).reshape(B, Sq, Hq, Dh), 0, 2, 1, 3)
    k = jnp.repeat(k_cache, rep, axis=1)
    v = jnp.repeat(v_cache, rep, axis=1)
    scores = jnp.einsum("bhqd,bhkd->bhqk", q, k) * (Dh ** -0.5)
    p = _softmax(scores, axis=-1)
    o = jnp.einsum("bhqk,bhkd->bhqd", p, v)
    return (lambda x, *d: x.transpose(*d))(o, 0, 2, 1, 3).reshape(B, Sq, Hq * Dh) @ wo
```

```python
import functools
import jax
import jax.numpy as jnp
from jax import lax
import jax.experimental.pallas as pl
import jax.experimental.pallas.tpu as pltpu

B, SQ, D = 32, 16, 1024
HQ, HKV, SK, DH = 32, 4, 2048, 128
REP = HQ // HKV
JB = 8
NJ = B // JB
GW = REP * DH
U = 1
NSLOT = 8
NITEM = HKV * B // U
SCALE = (DH ** -0.5) * 1.4426950408889634


def _kernel(x_hbm, k_hbm, v_hbm, wq_hbm, wo_hbm, out_hbm,
            x_v, wq_v, wo_v, kbuf, vbuf, q_scr, o_scr, acc_scr, out_v,
            ksem, vsem, wqsem, wosem, xsem, osem):

    def k_copy(i):
        slot = i % NSLOT
        return pltpu.make_async_copy(k_hbm.at[pl.ds((i % (B // U)) * U, U), i // (B // U)], kbuf.at[slot], ksem.at[slot])

    def v_copy(i):
        slot = i % NSLOT
        return pltpu.make_async_copy(v_hbm.at[pl.ds((i % (B // U)) * U, U), i // (B // U)], vbuf.at[slot], vsem.at[slot])

    def wq_copy(g):
        return pltpu.make_async_copy(wq_hbm.at[:, pl.ds(g * GW, GW)], wq_v.at[g], wqsem.at[g])

    def wo_copy(g):
        return pltpu.make_async_copy(wo_hbm.at[pl.ds(g * GW, GW), :], wo_v.at[g], wosem.at[g])

    def out_copy(j):
        return pltpu.make_async_copy(out_v.at[j], out_hbm.at[pl.ds(j * JB * SQ, JB * SQ), :], osem.at[j])

    x_copy = pltpu.make_async_copy(x_hbm, x_v, xsem.at[0])
    x_copy.start()
    wq_copy(0).start()
    for i in range(NSLOT):
        k_copy(i).start()
        v_copy(i).start()
        if i == 1:
            wo_copy(0).start()
    x_copy.wait()

    def superstep(ss, _):
        g = ss // NJ
        j = ss % NJ

        @pl.when(j == 0)
        def _():
            wq_copy(g).wait()

            @pl.when(g + 1 < HKV)
            def _():
                wq_copy(g + 1).start()
                wo_copy(g + 1).start()

        xr = x_v[pl.ds(pl.multiple_of(j * JB * SQ, JB * SQ), JB * SQ), :]
        q = jnp.dot(xr, wq_v[g], preferred_element_type=jnp.float32)
        q_scr[...] = (q * SCALE).astype(jnp.bfloat16)

        def attn(bp, _):
            i = g * (B // U) + j * (JB // U) + bp
            slot = i % NSLOT
            k_copy(i).wait()
            v_copy(i).wait()
            r0s = [pl.multiple_of((bp * U + u) * SQ, SQ) for u in range(U)]
            ss_ = []
            for u in range(U):
                qh = jnp.concatenate(
                    [q_scr[pl.ds(r0s[u], SQ), r * DH:(r + 1) * DH] for r in range(REP)], axis=0)
                ss_.append(lax.dot_general(qh, kbuf[slot, u], (((1,), (1,)), ((), ())),
                                           preferred_element_type=jnp.float32))
            for u in range(U):
                s = ss_[u]
                m = jnp.max(s, axis=1, keepdims=True)
                p = jnp.exp2(s - m)
                l = jnp.sum(p, axis=1, keepdims=True)
                o = jnp.dot(p.astype(jnp.bfloat16), vbuf[slot, u], preferred_element_type=jnp.float32)
                o = (o / l).astype(jnp.bfloat16)
                for r in range(REP):
                    o_scr[pl.ds(r0s[u], SQ), r * DH:(r + 1) * DH] = o[r * SQ:(r + 1) * SQ, :]

            @pl.when(i + NSLOT < NITEM)
            def _():
                k_copy(i + NSLOT).start()
                v_copy(i + NSLOT).start()
            return 0

        lax.fori_loop(0, JB // U, attn, 0)

        @pl.when(j == 0)
        def _():
            wo_copy(g).wait()

        part = jnp.dot(o_scr[...], wo_v[g], preferred_element_type=jnp.float32)

        @pl.when(g == 0)
        def _():
            acc_scr[j] = part

        @pl.when(jnp.logical_and(g > 0, g < HKV - 1))
        def _():
            acc_scr[j] += part

        @pl.when(g == HKV - 1)
        def _():
            out_v[j] = (acc_scr[j] + part).astype(jnp.bfloat16)
            out_copy(j).start()
        return 0

    lax.fori_loop(0, HKV * NJ, superstep, 0)
    for j in range(NJ):
        out_copy(j).wait()


@jax.jit
def pallas_standalone__gqa_block_cached__sampling_kernel(x, k_cache, v_cache, wq, wo):
    any_ = pl.BlockSpec(memory_space=pl.ANY)
    bf = jnp.bfloat16
    out = pl.pallas_call(
        _kernel,
        in_specs=[any_] * 5,
        out_specs=any_,
        out_shape=jax.ShapeDtypeStruct((B * SQ, D), bf),
        scratch_shapes=[
            pltpu.VMEM((B * SQ, D), bf),
            pltpu.VMEM((HKV, D, GW), bf),
            pltpu.VMEM((HKV, GW, D), bf),
            pltpu.VMEM((NSLOT, U, SK, DH), bf),
            pltpu.VMEM((NSLOT, U, SK, DH), bf),
            pltpu.VMEM((JB * SQ, GW), bf),
            pltpu.VMEM((JB * SQ, GW), bf),
            pltpu.VMEM((NJ, JB * SQ, D), jnp.float32),
            pltpu.VMEM((NJ, JB * SQ, D), bf),
            pltpu.SemaphoreType.DMA((NSLOT,)),
            pltpu.SemaphoreType.DMA((NSLOT,)),
            pltpu.SemaphoreType.DMA((HKV,)),
            pltpu.SemaphoreType.DMA((HKV,)),
            pltpu.SemaphoreType.DMA((1,)),
            pltpu.SemaphoreType.DMA((NJ,)),
        ],
        compiler_params=pltpu.CompilerParams(vmem_limit_bytes=100 * 2**20),
    )(x.reshape(B * SQ, D), k_cache, v_cache, wq, wo)
    return out.reshape(B, SQ, D)
```

```python
import jax
import jax.numpy as jnp
from jax import lax
import jax.experimental.pallas as pl
import jax.experimental.pallas.tpu as pltpu

B, SQ, D = 32, 16, 1024
HQ, HKV, SK, DH = 32, 4, 2048, 128
REP = HQ // HKV
GW = REP * DH
UB = 4
UM = UB * SQ
NRU = B // UB
NUNIT = HKV * NRU
PW = D // UB
QM = 128
NQC = B * SQ // QM
NSLOT = 8
NITEM = HKV * B
NPRE = 7
SKIPS = (6, 14, 22)
KV_PIECES = (128,) + (192,) * 10
KV_QUEUES = (0, 1, 1)
W_ROWS = 32
W_QUEUES = (0, 1)
N_INIT = 88
N_INIT_Q0 = 48
SCALE = (DH ** -0.5) * 1.4426950408889634


def _cut(sizes):
    out, o = [], 0
    for n in sizes:
        out.append((o, n))
        o += n
    return out


def _rows(r0, r1, step):
    return [(o, min(step, r1 - o)) for o in range(r0, r1, step)]


def _kernel(x_hbm, k_hbm, v_hbm, wq_hbm, wo_hbm, out_hbm,
            x_v, wq_v, wo_v, kbuf, vbuf, q_scr, o_scr, acc_scr, out_v,
            ksem, vsem, wqsem, wosem, osem):

    def start(copies, queues, first=0):
        for t, c in enumerate(copies):
            c.start(priority=queues[(first + t) % len(queues)])

    def kv_copies(i):
        slot = i % NSLOT
        b = i % B
        g = i // B
        return [pltpu.make_async_copy(src.at[b, g, pl.ds(o, n)], buf.at[slot, pl.ds(o, n)], sem.at[slot])
                for src, buf, sem in ((k_hbm, kbuf, ksem), (v_hbm, vbuf, vsem))
                for o, n in _cut(KV_PIECES)]

    def kv_wait(i):
        slot = i % NSLOT
        pltpu.make_async_copy(kbuf.at[slot], kbuf.at[slot], ksem.at[slot]).wait()
        pltpu.make_async_copy(vbuf.at[slot], vbuf.at[slot], vsem.at[slot]).wait()

    def out_start(r0, r1, sem):
        start([pltpu.make_async_copy(out_v.at[pl.ds(o, n)], out_hbm.at[pl.ds(o, n)], sem)
               for o, n in _rows(r0, r1, W_ROWS)], W_QUEUES)

    def out_wait(r0, r1, sem):
        pltpu.make_async_copy(out_v.at[pl.ds(r0, r1 - r0)], out_v.at[pl.ds(r0, r1 - r0)], sem).wait()

    def o_proj(u, par, c0, ncol):
        g = u // NRU
        ju = u % NRU
        part = jnp.dot(o_scr[par], wo_v[g, :, pl.ds(c0, ncol)], preferred_element_type=jnp.float32)
        tot = acc_scr[ju, :, pl.ds(c0, ncol)] + part
        acc_scr[ju, :, pl.ds(c0, ncol)] = tot
        out_v[pl.ds(pl.multiple_of(ju * UM, UM), UM), pl.ds(c0, ncol)] = tot.astype(jnp.bfloat16)

    def load_kv(buf, slot):
        return pltpu.bitcast(buf.bitcast(jnp.uint32)[slot], jnp.bfloat16)

    def prefetch(i):
        n = i + NPRE
        go = n < NITEM + len(SKIPS)
        for s in SKIPS:
            n = n - (i >= s).astype(jnp.int32)
            go = jnp.logical_and(go, i != s)

        @pl.when(jnp.logical_and(go, n < NITEM))
        def _():
            start(kv_copies(n), KV_QUEUES)

    def attend(i, oslices):
        g = i // B
        u = i // UB
        par = u % 2
        pos = i % UB
        slot = i % NSLOT
        rq = pl.multiple_of((i % B) * SQ, SQ)
        qh = jnp.concatenate([q_scr[g, pl.ds(rq, SQ), r * DH:(r + 1) * DH] for r in range(REP)], axis=0)
        s = lax.dot_general(qh, load_kv(kbuf, slot), (((1,), (1,)), ((), ())),
                            preferred_element_type=jnp.float32)
        if oslices:
            ncol = oslices * PW
            o_proj(jnp.maximum(u - 1, 0), 1 - par, pl.multiple_of(pos * ncol, ncol), ncol)
        m = jnp.max(s, axis=1, keepdims=True)
        p = jnp.exp2(s - m)
        l = jnp.sum(p, axis=1, keepdims=True)
        o = jnp.dot(p.astype(jnp.bfloat16), load_kv(vbuf, slot), preferred_element_type=jnp.float32)
        o = (o / l).astype(jnp.bfloat16)
        ro = pl.multiple_of(pos * SQ, SQ)
        for r in range(REP):
            o_scr[par, pl.ds(ro, SQ), r * DH:(r + 1) * DH] = o[r * SQ:(r + 1) * SQ, :]

    copies = [pltpu.make_async_copy(x_hbm.at[pl.ds(o, n)], x_v.at[pl.ds(o, n)], wqsem.at[0])
              for o, n in _rows(0, B * SQ, W_ROWS)]
    for g in range(HKV):
        copies += [pltpu.make_async_copy(wq_hbm.at[pl.ds(o, n), pl.ds(g * GW, GW)],
                                         wq_v.at[g, pl.ds(o, n)], wqsem.at[g])
                   for o, n in _rows(0, D, W_ROWS)]
    for g in range(HKV):
        copies += [pltpu.make_async_copy(wo_hbm.at[pl.ds(g * GW + o, n)],
                                         wo_v.at[g, pl.ds(o, n)], wosem.at[min(g, 1)])
                   for o, n in _rows(0, GW, W_ROWS)]
    for i in range(NPRE):
        copies += kv_copies(i)
    nchunk = HKV * NQC
    per = -(-(len(copies) - N_INIT) // (nchunk - 1))

    start(copies[:N_INIT_Q0], (0,))
    start(copies[N_INIT_Q0:N_INIT], W_QUEUES, N_INIT_Q0)
    o_scr[1] = jnp.zeros(o_scr.shape[1:], o_scr.dtype)
    acc_scr[...] = jnp.zeros(acc_scr.shape, acc_scr.dtype)

    def q_chunk(c, _):
        def batches(lo, hi):
            first = N_INIT + lo * per
            if first >= len(copies):
                return
            if hi - lo == 1:
                start(copies[first:first + per], W_QUEUES, first)
                return
            mid = (lo + hi) // 2
            pl.when(c - 1 < mid)(lambda: batches(lo, mid))
            pl.when(c - 1 >= mid)(lambda: batches(mid, hi))

        pl.when(c > 0)(lambda: batches(0, nchunk - 1))
        g = c // NQC
        j = c % NQC

        @pl.when(c == 0)
        def _():
            pltpu.make_async_copy(x_v, x_v, wqsem.at[0]).wait()

        @pl.when(j == 0)
        def _():
            pltpu.make_async_copy(wq_v.at[g], wq_v.at[g], wqsem.at[g]).wait()

        r0 = pl.multiple_of(j * QM, QM)
        q = jnp.dot(x_v[pl.ds(r0, QM), :], wq_v[g], preferred_element_type=jnp.float32)
        q_scr[g, pl.ds(r0, QM), :] = (q * SCALE).astype(jnp.bfloat16)
        return 0

    lax.fori_loop(0, nchunk, q_chunk, 0)
    pltpu.make_async_copy(wo_v.at[0], wo_v.at[0], wosem.at[0]).wait()

    def step(i, _):
        @pl.when(i == B)
        def _():
            pltpu.make_async_copy(wo_v.at[pl.ds(1, HKV - 1)], wo_v.at[pl.ds(1, HKV - 1)], wosem.at[1]).wait()

        prefetch(i)
        kv_wait(i)
        attend(i, 1)
        return 0

    lax.fori_loop(0, NITEM - UB, step, 0)

    def step_wide(i, _):
        kv_wait(i)
        attend(i, 2)
        return 0

    lax.fori_loop(NITEM - UB, NITEM - 2, step_wide, 0)
    kv_wait(NITEM - 2)
    attend(jnp.int32(NITEM - 2), 0)
    kv_wait(NITEM - 1)
    done = (NRU - 1) * UM
    out_start(0, done, osem.at[0])
    attend(jnp.int32(NITEM - 1), 0)
    o_proj(NUNIT - 1, (NUNIT - 1) % 2, 0, D)
    out_start(done, B * SQ, osem.at[1])
    out_wait(0, done, osem.at[0])
    out_wait(done, B * SQ, osem.at[1])


@jax.jit
def pallas_standalone__gqa_block_cached__sampling_kernel(
    x: jax.Array,
    k_cache: jax.Array,
    v_cache: jax.Array,
    wq: jax.Array,
    wo: jax.Array,
):
    bf = jnp.bfloat16
    hbm = pl.BlockSpec(memory_space=pl.ANY)
    out = pl.pallas_call(
        _kernel,
        in_specs=[hbm] * 5,
        out_specs=hbm,
        out_shape=jax.ShapeDtypeStruct((B * SQ, D), bf),
        scratch_shapes=[
            pltpu.VMEM((B * SQ, D), bf),
            pltpu.VMEM((HKV, D, GW), bf),
            pltpu.VMEM((HKV, GW, D), bf),
            pltpu.VMEM((NSLOT, SK, DH), bf),
            pltpu.VMEM((NSLOT, SK, DH), bf),
            pltpu.VMEM((HKV, B * SQ, GW), bf),
            pltpu.VMEM((2, UM, GW), bf),
            pltpu.VMEM((NRU, UM, D), jnp.float32),
            pltpu.VMEM((B * SQ, D), bf),
            pltpu.SemaphoreType.DMA((NSLOT,)),
            pltpu.SemaphoreType.DMA((NSLOT,)),
            pltpu.SemaphoreType.DMA((HKV,)),
            pltpu.SemaphoreType.DMA((2,)),
            pltpu.SemaphoreType.DMA((2,)),
        ],
        compiler_params=pltpu.CompilerParams(vmem_limit_bytes=64 * 2**20, disable_bounds_checks=True),
    )(x.reshape(B * SQ, D), k_cache, v_cache, wq, wo)
    return out.reshape(B, SQ, D)
```

```python
import jax
import jax.numpy as jnp
from jax import lax
import jax.experimental.pallas as pl
import jax.experimental.pallas.tpu as pltpu

B, SQ, D = 32, 16, 1024
HQ, HKV, SK, DH = 32, 4, 2048, 128
REP = HQ // HKV
GW = REP * DH
UB = 4
UM = UB * SQ
NRU = B // UB
NUNIT = HKV * NRU
PW = D // UB
QM = 128
NQC = B * SQ // QM
NSLOT = 8
NITEM = HKV * B
NPRE = 7
SKIPS = (6, 14, 22)
KV_PIECES = (128,) + (192,) * 10
KV_QUEUES = (0, 1, 1)
N_ORDERED = 3
W_ROWS = 32
W_QUEUES = (0, 1)
N_INIT = 88
N_INIT_Q0 = 48
SCALE = (DH ** -0.5) * 1.4426950408889634


def _cut(sizes):
    out, o = [], 0
    for n in sizes:
        out.append((o, n))
        o += n
    return out


def _rows(r0, r1, step):
    return [(o, min(step, r1 - o)) for o in range(r0, r1, step)]


def _kernel(x_hbm, k_hbm, v_hbm, wq_hbm, wo_hbm, out_hbm,
            x_v, wq_v, wo_v, kbuf, vbuf, q_scr, o_scr, acc_scr, out_v,
            ksem, vsem, wqsem, wosem, osem):

    def start(copies, queues, first=0):
        for t, c in enumerate(copies):
            c.start(priority=queues[(first + t) % len(queues)])

    def kv_copies(i):
        slot = i % NSLOT
        b = i % B
        g = i // B
        return [pltpu.make_async_copy(src.at[b, g, pl.ds(o, n)], buf.at[slot, pl.ds(o, n)], sem.at[slot])
                for src, buf, sem in ((k_hbm, kbuf, ksem), (v_hbm, vbuf, vsem))
                for o, n in _cut(KV_PIECES)]

    def kv_wait(i):
        slot = i % NSLOT
        pltpu.make_async_copy(kbuf.at[slot], kbuf.at[slot], ksem.at[slot]).wait()
        pltpu.make_async_copy(vbuf.at[slot], vbuf.at[slot], vsem.at[slot]).wait()

    def out_start(r0, r1, sem):
        start([pltpu.make_async_copy(out_v.at[pl.ds(o, n)], out_hbm.at[pl.ds(o, n)], sem)
               for o, n in _rows(r0, r1, W_ROWS)], W_QUEUES)

    def out_wait(r0, r1, sem):
        pltpu.make_async_copy(out_v.at[pl.ds(r0, r1 - r0)], out_v.at[pl.ds(r0, r1 - r0)], sem).wait()

    def o_proj(u, par, c0, ncol):
        g = u // NRU
        ju = u % NRU
        part = jnp.dot(o_scr[par], wo_v[g, :, pl.ds(c0, ncol)], preferred_element_type=jnp.float32)
        tot = acc_scr[ju, :, pl.ds(c0, ncol)] + part
        acc_scr[ju, :, pl.ds(c0, ncol)] = tot
        out_v[pl.ds(pl.multiple_of(ju * UM, UM), UM), pl.ds(c0, ncol)] = tot.astype(jnp.bfloat16)

    def load_kv(buf, slot):
        return pltpu.bitcast(buf.bitcast(jnp.uint32)[slot], jnp.bfloat16)

    def prefetch(i):
        n = i + NPRE
        go = n >= NPRE
        for s in SKIPS:
            n = n - (i >= s).astype(jnp.int32)
            go = jnp.logical_and(go, i != s)

        @pl.when(jnp.logical_and(go, n < NITEM - N_ORDERED))
        def _():
            start(kv_copies(n), KV_QUEUES)

        @pl.when(jnp.logical_and(go, jnp.logical_and(n >= NITEM - N_ORDERED, n < NITEM)))
        def _():
            start(kv_copies(n), (1,))

    def attend(i, oslices):
        g = i // B
        u = i // UB
        par = u % 2
        pos = i % UB
        slot = i % NSLOT
        rq = pl.multiple_of((i % B) * SQ, SQ)
        qh = jnp.concatenate([q_scr[g, pl.ds(rq, SQ), r * DH:(r + 1) * DH] for r in range(REP)], axis=0)
        s = lax.dot_general(qh, load_kv(kbuf, slot), (((1,), (1,)), ((), ())),
                            preferred_element_type=jnp.float32)
        if oslices:
            ncol = oslices * PW
            o_proj(jnp.maximum(u - 1, 0), 1 - par, pl.multiple_of(pos * ncol, ncol), ncol)
        m = jnp.max(s, axis=1, keepdims=True)
        p = jnp.exp2(s - m)
        l = jnp.sum(p, axis=1, keepdims=True)
        o = jnp.dot(p.astype(jnp.bfloat16), load_kv(vbuf, slot), preferred_element_type=jnp.float32)
        o = (o / l).astype(jnp.bfloat16)
        ro = pl.multiple_of(pos * SQ, SQ)
        for r in range(REP):
            o_scr[par, pl.ds(ro, SQ), r * DH:(r + 1) * DH] = o[r * SQ:(r + 1) * SQ, :]

    copies = [pltpu.make_async_copy(x_hbm.at[pl.ds(o, n)], x_v.at[pl.ds(o, n)], wqsem.at[0])
              for o, n in _rows(0, B * SQ, W_ROWS)]
    for g in range(HKV):
        copies += [pltpu.make_async_copy(wq_hbm.at[pl.ds(o, n), pl.ds(g * GW, GW)],
                                         wq_v.at[g, pl.ds(o, n)], wqsem.at[g])
                   for o, n in _rows(0, D, W_ROWS)]
    for g in range(HKV):
        copies += [pltpu.make_async_copy(wo_hbm.at[pl.ds(g * GW + o, n)],
                                         wo_v.at[g, pl.ds(o, n)], wosem.at[min(g, 1)])
                   for o, n in _rows(0, GW, W_ROWS)]
    for i in range(NPRE):
        copies += kv_copies(i)
    nchunk = HKV * NQC
    per = -(-(len(copies) - N_INIT) // (nchunk - 1))

    start(copies[:N_INIT_Q0], (0,))
    start(copies[N_INIT_Q0:N_INIT], W_QUEUES, N_INIT_Q0)
    o_scr[1] = jnp.zeros(o_scr.shape[1:], o_scr.dtype)
    acc_scr[...] = jnp.zeros(acc_scr.shape, acc_scr.dtype)

    def q_chunk(c, _):
        def batches(lo, hi):
            first = N_INIT + lo * per
            if first >= len(copies):
                return
            if hi - lo == 1:
                start(copies[first:first + per], W_QUEUES, first)
                return
            mid = (lo + hi) // 2
            pl.when(c - 1 < mid)(lambda: batches(lo, mid))
            pl.when(c - 1 >= mid)(lambda: batches(mid, hi))

        pl.when(c > 0)(lambda: batches(0, nchunk - 1))
        g = c // NQC
        j = c % NQC

        @pl.when(c == 0)
        def _():
            pltpu.make_async_copy(x_v, x_v, wqsem.at[0]).wait()

        @pl.when(j == 0)
        def _():
            pltpu.make_async_copy(wq_v.at[g], wq_v.at[g], wqsem.at[g]).wait()

        r0 = pl.multiple_of(j * QM, QM)
        q = jnp.dot(x_v[pl.ds(r0, QM), :], wq_v[g], preferred_element_type=jnp.float32)
        q_scr[g, pl.ds(r0, QM), :] = (q * SCALE).astype(jnp.bfloat16)
        return 0

    lax.fori_loop(0, nchunk, q_chunk, 0)
    pltpu.make_async_copy(wo_v.at[0], wo_v.at[0], wosem.at[0]).wait()

    def step(i, _):
        @pl.when(i == B)
        def _():
            pltpu.make_async_copy(wo_v.at[pl.ds(1, HKV - 1)], wo_v.at[pl.ds(1, HKV - 1)], wosem.at[1]).wait()

        prefetch(i)
        kv_wait(i)
        attend(i, 1)
        return 0

    lax.fori_loop(0, NITEM - UB, step, 0)

    def step_wide(i, _):
        kv_wait(i)
        attend(i, 2)
        return 0

    lax.fori_loop(NITEM - UB, NITEM - 2, step_wide, 0)
    kv_wait(NITEM - 2)
    attend(jnp.int32(NITEM - 2), 0)
    kv_wait(NITEM - 1)
    done = (NRU - 1) * UM
    out_start(0, done, osem.at[0])
    attend(jnp.int32(NITEM - 1), 0)
    half = D // 2
    for t in range(2):
        o_proj(NUNIT - 1, (NUNIT - 1) % 2, t * half, half)
        pltpu.make_async_copy(out_v.at[pl.ds(done, UM), pl.ds(t * half, half)],
                              out_hbm.at[pl.ds(done, UM), pl.ds(t * half, half)],
                              osem.at[1]).start(priority=t)
    out_wait(0, done, osem.at[0])
    out_wait(done, B * SQ, osem.at[1])


@jax.jit
def pallas_standalone__gqa_block_cached__sampling_kernel(
    x: jax.Array,
    k_cache: jax.Array,
    v_cache: jax.Array,
    wq: jax.Array,
    wo: jax.Array,
):
    bf = jnp.bfloat16
    hbm = pl.BlockSpec(memory_space=pl.ANY)
    out = pl.pallas_call(
        _kernel,
        in_specs=[hbm] * 5,
        out_specs=hbm,
        out_shape=jax.ShapeDtypeStruct((B * SQ, D), bf),
        scratch_shapes=[
            pltpu.VMEM((B * SQ, D), bf),
            pltpu.VMEM((HKV, D, GW), bf),
            pltpu.VMEM((HKV, GW, D), bf),
            pltpu.VMEM((NSLOT, SK, DH), bf),
            pltpu.VMEM((NSLOT, SK, DH), bf),
            pltpu.VMEM((HKV, B * SQ, GW), bf),
            pltpu.VMEM((2, UM, GW), bf),
            pltpu.VMEM((NRU, UM, D), jnp.float32),
            pltpu.VMEM((B * SQ, D), bf),
            pltpu.SemaphoreType.DMA((NSLOT,)),
            pltpu.SemaphoreType.DMA((NSLOT,)),
            pltpu.SemaphoreType.DMA((HKV,)),
            pltpu.SemaphoreType.DMA((2,)),
            pltpu.SemaphoreType.DMA((2,)),
        ],
        compiler_params=pltpu.CompilerParams(
            vmem_limit_bytes=64 * 2**20,
            disable_bounds_checks=True,
            disable_semaphore_checks=True,
        ),
    )(x.reshape(B * SQ, D), k_cache, v_cache, wq, wo)
    return out.reshape(B, SQ, D)
```

```python
import jax
import jax.numpy as jnp
from jax import lax
import jax.experimental.pallas as pl
import jax.experimental.pallas.tpu as pltpu

B, SQ, D = 32, 16, 1024
HQ, HKV, SK, DH = 32, 4, 2048, 128
REP = HQ // HKV
GW = REP * DH
HG = REP // 2
UB = 4
UM = UB * SQ
NRU = B // UB
NUNIT = HKV * NRU
PW = D // UB
QM = 128
NQC = B * SQ // QM
NSLOT = 8
NITEM = HKV * B
NPRE = 7
SKIPS = (6, 14, 22)
KV_PIECES = (128,) + (192,) * 10
KV_QUEUES = (0, 1, 1)
N_ORDERED = 3
W_ROWS = 32
W_QUEUES = (0, 1)
N_INIT = 88
N_INIT_Q0 = 48
SCALE = (DH ** -0.5) * 1.4426950408889634


def _cut(sizes):
    out, o = [], 0
    for n in sizes:
        out.append((o, n))
        o += n
    return out


def _rows(r0, r1, step):
    return [(o, min(step, r1 - o)) for o in range(r0, r1, step)]


def _kernel(x_hbm, k_hbm, v_hbm, wq_hbm, wo_hbm, out_hbm,
            x_v, wq_v, wo_v, kbuf, vbuf, q_scr, o_scr, acc_scr, out_v,
            ksem, vsem, wqsem, wosem, osem):

    def start(copies, queues, first=0):
        for t, c in enumerate(copies):
            c.start(priority=queues[(first + t) % len(queues)])

    def kv_copies(i):
        slot = i % NSLOT
        b = i % B
        g = i // B
        return [pltpu.make_async_copy(src.at[b, g, pl.ds(o, n)], buf.at[slot, pl.ds(o, n)], sem.at[slot])
                for src, buf, sem in ((k_hbm, kbuf, ksem), (v_hbm, vbuf, vsem))
                for o, n in _cut(KV_PIECES)]

    def kv_wait(i):
        slot = i % NSLOT
        pltpu.make_async_copy(kbuf.at[slot], kbuf.at[slot], ksem.at[slot]).wait()
        pltpu.make_async_copy(vbuf.at[slot], vbuf.at[slot], vsem.at[slot]).wait()

    def out_start(r0, r1, sem):
        start([pltpu.make_async_copy(out_v.at[pl.ds(o, n)], out_hbm.at[pl.ds(o, n)], sem)
               for o, n in _rows(r0, r1, W_ROWS)], W_QUEUES)

    def out_wait(r0, r1, sem):
        pltpu.make_async_copy(out_v.at[pl.ds(r0, r1 - r0)], out_v.at[pl.ds(r0, r1 - r0)], sem).wait()

    def o_proj(u, par, c0, ncol):
        g = u // NRU
        ju = u % NRU
        part = jnp.dot(o_scr[par], wo_v[g, :, pl.ds(c0, ncol)], preferred_element_type=jnp.float32)
        tot = acc_scr[ju, :, pl.ds(c0, ncol)] + part
        acc_scr[ju, :, pl.ds(c0, ncol)] = tot
        out_v[pl.ds(pl.multiple_of(ju * UM, UM), UM), pl.ds(c0, ncol)] = tot.astype(jnp.bfloat16)

    def load_kv(buf, slot):
        return pltpu.bitcast(buf.bitcast(jnp.uint32)[slot], jnp.bfloat16)

    def prefetch(i):
        n = i + NPRE
        go = n >= NPRE
        for s in SKIPS:
            n = n - (i >= s).astype(jnp.int32)
            go = jnp.logical_and(go, i != s)

        @pl.when(jnp.logical_and(go, n < NITEM - N_ORDERED))
        def _():
            start(kv_copies(n), KV_QUEUES)

        @pl.when(jnp.logical_and(go, jnp.logical_and(n >= NITEM - N_ORDERED, n < NITEM)))
        def _():
            start(kv_copies(n), (1,))

    def attend(i, oslices):
        g = i // B
        u = i // UB
        par = u % 2
        pos = i % UB
        slot = i % NSLOT
        rq = pl.multiple_of((i % B) * SQ, SQ)
        ro = pl.multiple_of(pos * SQ, SQ)
        k = load_kv(kbuf, slot)
        v = load_kv(vbuf, slot)
        scores = []
        for h in range(2):
            qh = jnp.concatenate([q_scr[g, pl.ds(rq, SQ), r * DH:(r + 1) * DH]
                                  for r in range(h * HG, (h + 1) * HG)], axis=0)
            scores.append(lax.dot_general(qh, k, (((1,), (1,)), ((), ())),
                                          preferred_element_type=jnp.float32))
            if h == 0 and oslices:
                ncol = oslices * PW
                o_proj(jnp.maximum(u - 1, 0), 1 - par, pl.multiple_of(pos * ncol, ncol), ncol)
        for h in range(2):
            s = scores[h]
            m = jnp.max(s, axis=1, keepdims=True)
            p = jnp.exp2(s - m)
            l = jnp.sum(p, axis=1, keepdims=True)
            o = jnp.dot(p.astype(jnp.bfloat16), v, preferred_element_type=jnp.float32)
            o = (o / l).astype(jnp.bfloat16)
            for r in range(HG):
                c = (h * HG + r) * DH
                o_scr[par, pl.ds(ro, SQ), c:c + DH] = o[r * SQ:(r + 1) * SQ, :]

    copies = [pltpu.make_async_copy(x_hbm.at[pl.ds(o, n)], x_v.at[pl.ds(o, n)], wqsem.at[0])
              for o, n in _rows(0, B * SQ, W_ROWS)]
    for g in range(HKV):
        copies += [pltpu.make_async_copy(wq_hbm.at[pl.ds(o, n), pl.ds(g * GW, GW)],
                                         wq_v.at[g, pl.ds(o, n)], wqsem.at[g])
                   for o, n in _rows(0, D, W_ROWS)]
    for g in range(HKV):
        copies += [pltpu.make_async_copy(wo_hbm.at[pl.ds(g * GW + o, n)],
                                         wo_v.at[g, pl.ds(o, n)], wosem.at[min(g, 1)])
                   for o, n in _rows(0, GW, W_ROWS)]
    for i in range(NPRE):
        copies += kv_copies(i)
    nchunk = HKV * NQC
    per = -(-(len(copies) - N_INIT) // (nchunk - 1))

    start(copies[:N_INIT_Q0], (0,))
    start(copies[N_INIT_Q0:N_INIT], W_QUEUES, N_INIT_Q0)
    o_scr[1] = jnp.zeros(o_scr.shape[1:], o_scr.dtype)
    acc_scr[...] = jnp.zeros(acc_scr.shape, acc_scr.dtype)

    def q_chunk(c, _):
        def batches(lo, hi):
            first = N_INIT + lo * per
            if first >= len(copies):
                return
            if hi - lo == 1:
                start(copies[first:first + per], W_QUEUES, first)
                return
            mid = (lo + hi) // 2
            pl.when(c - 1 < mid)(lambda: batches(lo, mid))
            pl.when(c - 1 >= mid)(lambda: batches(mid, hi))

        pl.when(c > 0)(lambda: batches(0, nchunk - 1))
        g = c // NQC
        j = c % NQC

        @pl.when(c == 0)
        def _():
            pltpu.make_async_copy(x_v, x_v, wqsem.at[0]).wait()

        @pl.when(j == 0)
        def _():
            pltpu.make_async_copy(wq_v.at[g], wq_v.at[g], wqsem.at[g]).wait()

        r0 = pl.multiple_of(j * QM, QM)
        q = jnp.dot(x_v[pl.ds(r0, QM), :], wq_v[g], preferred_element_type=jnp.float32)
        q_scr[g, pl.ds(r0, QM), :] = (q * SCALE).astype(jnp.bfloat16)
        return 0

    lax.fori_loop(0, nchunk, q_chunk, 0)
    pltpu.make_async_copy(wo_v.at[0], wo_v.at[0], wosem.at[0]).wait()

    def step(i, _):
        @pl.when(i == B)
        def _():
            pltpu.make_async_copy(wo_v.at[pl.ds(1, HKV - 1)], wo_v.at[pl.ds(1, HKV - 1)], wosem.at[1]).wait()

        prefetch(i)
        kv_wait(i)
        attend(i, 1)
        return 0

    lax.fori_loop(0, NITEM - UB, step, 0)

    def step_wide(i, _):
        kv_wait(i)
        attend(i, 2)
        return 0

    lax.fori_loop(NITEM - UB, NITEM - 2, step_wide, 0)
    kv_wait(NITEM - 2)
    attend(jnp.int32(NITEM - 2), 0)
    kv_wait(NITEM - 1)
    done = (NRU - 1) * UM
    out_start(0, done, osem.at[0])
    attend(jnp.int32(NITEM - 1), 0)
    half = D // 2
    for t in range(2):
        o_proj(NUNIT - 1, (NUNIT - 1) % 2, t * half, half)
        pltpu.make_async_copy(out_v.at[pl.ds(done, UM), pl.ds(t * half, half)],
                              out_hbm.at[pl.ds(done, UM), pl.ds(t * half, half)],
                              osem.at[1]).start(priority=t)
    out_wait(0, done, osem.at[0])
    out_wait(done, B * SQ, osem.at[1])


@jax.jit
def pallas_standalone__gqa_block_cached__sampling_kernel(
    x: jax.Array,
    k_cache: jax.Array,
    v_cache: jax.Array,
    wq: jax.Array,
    wo: jax.Array,
):
    bf = jnp.bfloat16
    hbm = pl.BlockSpec(memory_space=pl.ANY)
    out = pl.pallas_call(
        _kernel,
        in_specs=[hbm] * 5,
        out_specs=hbm,
        out_shape=jax.ShapeDtypeStruct((B * SQ, D), bf),
        scratch_shapes=[
            pltpu.VMEM((B * SQ, D), bf),
            pltpu.VMEM((HKV, D, GW), bf),
            pltpu.VMEM((HKV, GW, D), bf),
            pltpu.VMEM((NSLOT, SK, DH), bf),
            pltpu.VMEM((NSLOT, SK, DH), bf),
            pltpu.VMEM((HKV, B * SQ, GW), bf),
            pltpu.VMEM((2, UM, GW), bf),
            pltpu.VMEM((NRU, UM, D), jnp.float32),
            pltpu.VMEM((B * SQ, D), bf),
            pltpu.SemaphoreType.DMA((NSLOT,)),
            pltpu.SemaphoreType.DMA((NSLOT,)),
            pltpu.SemaphoreType.DMA((HKV,)),
            pltpu.SemaphoreType.DMA((2,)),
            pltpu.SemaphoreType.DMA((2,)),
        ],
        compiler_params=pltpu.CompilerParams(
            vmem_limit_bytes=64 * 2**20,
            disable_bounds_checks=True,
            disable_semaphore_checks=True,
        ),
    )(x.reshape(B * SQ, D), k_cache, v_cache, wq, wo)
    return out.reshape(B, SQ, D)
```

```python
import jax
import jax.numpy as jnp
from jax import lax
import jax.experimental.pallas as pl
import jax.experimental.pallas.tpu as pltpu

B, SQ, D = 32, 16, 1024
HQ, HKV, SK, DH = 32, 4, 2048, 128
REP = HQ // HKV
GW = REP * DH
HG = REP // 2
UB = 4
UM = UB * SQ
NRU = B // UB
NUNIT = HKV * NRU
PW = D // UB
QM = 128
NQC = B * SQ // QM
NSLOT = 8
NITEM = HKV * B
NPRE = 7
SKIPS = (6, 14, 22)
KV_PIECES = (128,) + (192,) * 10
KV_QUEUES = (0, 1, 1)
N_ORDERED = 3
W_ROWS = 32
W_QUEUES = (0, 1)
N_INIT = 88
N_INIT_Q0 = 48
SCALE = (DH ** -0.5) * 1.4426950408889634


def _cut(sizes):
    out, o = [], 0
    for n in sizes:
        out.append((o, n))
        o += n
    return out


def _rows(r0, r1, step):
    return [(o, min(step, r1 - o)) for o in range(r0, r1, step)]


def _kernel(x_hbm, k_hbm, v_hbm, wq_hbm, wo_hbm, out_hbm,
            xw_v, wo_v, kbuf, vbuf, q_scr, o_scr, acc_scr, out_v,
            ksem, vsem, wqsem, wosem, osem):

    def start(copies, queues, first=0):
        for t, c in enumerate(copies):
            c.start(priority=queues[(first + t) % len(queues)])

    def kv_copies(i):
        slot = i % NSLOT
        b = i % B
        g = i // B
        return [pltpu.make_async_copy(src.at[b, g, pl.ds(o, n)], buf.at[slot, pl.ds(o, n)], sem.at[slot])
                for src, buf, sem in ((k_hbm, kbuf, ksem), (v_hbm, vbuf, vsem))
                for o, n in _cut(KV_PIECES)]

    def kv_wait(i):
        slot = i % NSLOT
        pltpu.make_async_copy(kbuf.at[slot], kbuf.at[slot], ksem.at[slot]).wait()
        pltpu.make_async_copy(vbuf.at[slot], vbuf.at[slot], vsem.at[slot]).wait()

    def out_start(r0, r1, sem):
        start([pltpu.make_async_copy(out_v.at[pl.ds(o, n)], out_hbm.at[pl.ds(o, n)], sem)
               for o, n in _rows(r0, r1, W_ROWS)], W_QUEUES)

    def out_wait(r0, r1, sem):
        pltpu.make_async_copy(out_v.at[pl.ds(r0, r1 - r0)], out_v.at[pl.ds(r0, r1 - r0)], sem).wait()

    def o_proj(u, par, c0, ncol):
        g = u // NRU
        ju = u % NRU
        part = jnp.dot(o_scr[par], wo_v[g, :, pl.ds(c0, ncol)], preferred_element_type=jnp.float32)
        tot = acc_scr[ju, :, pl.ds(c0, ncol)] + part
        acc_scr[ju, :, pl.ds(c0, ncol)] = tot
        out_v[pl.ds(pl.multiple_of(ju * UM, UM), UM), pl.ds(c0, ncol)] = tot.astype(jnp.bfloat16)

    def prefetch(i):
        n = i + NPRE
        go = i != SKIPS[0]
        for s in SKIPS:
            n = n - (i >= s).astype(jnp.int32)
            go = jnp.logical_and(go, i != s)

        @pl.when(jnp.logical_and(go, n < NITEM - N_ORDERED))
        def _():
            start(kv_copies(n), KV_QUEUES)

        @pl.when(jnp.logical_and(go, jnp.logical_and(n >= NITEM - N_ORDERED, n < NITEM)))
        def _():
            start(kv_copies(n), (1,))

    def attend(i, oslices):
        g = i // B
        u = i // UB
        par = u % 2
        pos = i % UB
        slot = i % NSLOT
        rq = pl.multiple_of((i % B) * SQ, SQ)
        ro = pl.multiple_of(pos * SQ, SQ)
        k = kbuf[slot]
        v = vbuf[slot]
        scores = []
        for h in range(2):
            qh = jnp.concatenate([q_scr[g, pl.ds(rq, SQ), r * DH:(r + 1) * DH]
                                  for r in range(h * HG, (h + 1) * HG)], axis=0)
            scores.append(lax.dot_general(qh, k, (((1,), (1,)), ((), ())),
                                          preferred_element_type=jnp.float32))
            if h == 0 and oslices:
                ncol = oslices * PW
                o_proj(jnp.maximum(u - 1, 0), 1 - par, pl.multiple_of(pos * ncol, ncol), ncol)
        for h in range(2):
            s = scores[h]
            m = jnp.max(s, axis=1, keepdims=True)
            p = jnp.exp2(s - m)
            l = jnp.sum(p, axis=1, keepdims=True)
            o = jnp.dot(p.astype(jnp.bfloat16), v, preferred_element_type=jnp.float32)
            o = (o / l).astype(jnp.bfloat16)
            for r in range(HG):
                c = (h * HG + r) * DH
                o_scr[par, pl.ds(ro, SQ), c:c + DH] = o[r * SQ:(r + 1) * SQ, :]

    copies = [pltpu.make_async_copy(x_hbm.at[pl.ds(o, n)], xw_v.at[pl.ds(o, n)], wqsem.at[0])
              for o, n in _rows(0, B * SQ, W_ROWS)]
    for g in range(HKV):
        copies += [pltpu.make_async_copy(wq_hbm.at[pl.ds(o, n), pl.ds(g * GW, GW)],
                                         xw_v.at[pl.ds(B * SQ + g * D + o, n)], wqsem.at[g])
                   for o, n in _rows(0, D, W_ROWS)]
    for g in range(HKV):
        copies += [pltpu.make_async_copy(wo_hbm.at[pl.ds(g * GW + o, n)],
                                         wo_v.at[g, pl.ds(o, n)], wosem.at[min(g, 1)])
                   for o, n in _rows(0, GW, W_ROWS)]
    for i in range(NPRE):
        copies += kv_copies(i)
    nchunk = HKV * NQC
    per = -(-(len(copies) - N_INIT) // (nchunk - 1))

    start(copies[:N_INIT_Q0], (0,))
    start(copies[N_INIT_Q0:N_INIT], W_QUEUES, N_INIT_Q0)
    o_scr[1] = jnp.zeros(o_scr.shape[1:], o_scr.dtype)
    acc_scr[...] = jnp.zeros(acc_scr.shape, acc_scr.dtype)

    def q_chunk(c, _):
        def batches(lo, hi):
            first = N_INIT + lo * per
            if first >= len(copies):
                return
            if hi - lo == 1:
                start(copies[first:first + per], W_QUEUES, first)
                return
            mid = (lo + hi) // 2
            pl.when(c - 1 < mid)(lambda: batches(lo, mid))
            pl.when(c - 1 >= mid)(lambda: batches(mid, hi))

        pl.when(c > 0)(lambda: batches(0, nchunk - 1))
        g = c // NQC
        j = c % NQC

        w0 = pl.multiple_of(B * SQ + g * D, B * SQ)

        @pl.when(c == 0)
        def _():
            both = xw_v.at[pl.ds(0, B * SQ + D)]
            pltpu.make_async_copy(both, both, wqsem.at[0]).wait()

        @pl.when(jnp.logical_and(j == 0, c > 0))
        def _():
            slab = xw_v.at[pl.ds(w0, D)]
            pltpu.make_async_copy(slab, slab, wqsem.at[g]).wait()

        r0 = pl.multiple_of(j * QM, QM)
        q = jnp.dot(xw_v[pl.ds(r0, QM), :], xw_v[pl.ds(w0, D), :], preferred_element_type=jnp.float32)
        q_scr[g, pl.ds(r0, QM), :] = (q * SCALE).astype(jnp.bfloat16)
        return 0

    lax.fori_loop(0, nchunk, q_chunk, 0)
    pltpu.make_async_copy(wo_v.at[0], wo_v.at[0], wosem.at[0]).wait()

    def step(i, _):
        @pl.when(i == B)
        def _():
            pltpu.make_async_copy(wo_v.at[pl.ds(1, HKV - 1)], wo_v.at[pl.ds(1, HKV - 1)], wosem.at[1]).wait()

        prefetch(i)
        kv_wait(i)
        attend(i, 1)
        return 0

    lax.fori_loop(0, NITEM - UB, step, 0)

    def step_wide(i, _):
        kv_wait(i)
        attend(i, 2)
        return 0

    lax.fori_loop(NITEM - UB, NITEM - 2, step_wide, 0)
    kv_wait(NITEM - 2)
    attend(jnp.int32(NITEM - 2), 0)
    kv_wait(NITEM - 1)
    done = (NRU - 1) * UM
    out_start(0, done, osem.at[0])
    attend(jnp.int32(NITEM - 1), 0)
    half = D // 2
    for t in range(2):
        o_proj(NUNIT - 1, (NUNIT - 1) % 2, t * half, half)
        pltpu.make_async_copy(out_v.at[pl.ds(done, UM), pl.ds(t * half, half)],
                              out_hbm.at[pl.ds(done, UM), pl.ds(t * half, half)],
                              osem.at[1]).start(priority=t)
    out_wait(0, done, osem.at[0])
    out_wait(done, B * SQ, osem.at[1])


@jax.jit
def pallas_standalone__gqa_block_cached__sampling_kernel(
    x: jax.Array,
    k_cache: jax.Array,
    v_cache: jax.Array,
    wq: jax.Array,
    wo: jax.Array,
):
    bf = jnp.bfloat16
    hbm = pl.BlockSpec(memory_space=pl.ANY)
    out = pl.pallas_call(
        _kernel,
        in_specs=[hbm] * 5,
        out_specs=hbm,
        out_shape=jax.ShapeDtypeStruct((B * SQ, D), bf),
        scratch_shapes=[
            pltpu.VMEM((B * SQ + HKV * D, GW), bf),
            pltpu.VMEM((HKV, GW, D), bf),
            pltpu.VMEM((NSLOT, SK, DH), bf),
            pltpu.VMEM((NSLOT, SK, DH), bf),
            pltpu.VMEM((HKV, B * SQ, GW), bf),
            pltpu.VMEM((2, UM, GW), bf),
            pltpu.VMEM((NRU, UM, D), jnp.float32),
            pltpu.VMEM((B * SQ, D), bf),
            pltpu.SemaphoreType.DMA((NSLOT,)),
            pltpu.SemaphoreType.DMA((NSLOT,)),
            pltpu.SemaphoreType.DMA((HKV,)),
            pltpu.SemaphoreType.DMA((2,)),
            pltpu.SemaphoreType.DMA((2,)),
        ],
        compiler_params=pltpu.CompilerParams(
            vmem_limit_bytes=64 * 2**20,
            disable_bounds_checks=True,
            disable_semaphore_checks=True,
        ),
    )(x.reshape(B * SQ, D), k_cache, v_cache, wq, wo)
    return out.reshape(B, SQ, D)
```

```python
import jax
import jax.numpy as jnp
from jax import lax
import jax.experimental.pallas as pl
import jax.experimental.pallas.tpu as pltpu

B, SQ, D = 32, 16, 1024
HQ, HKV, SK, DH = 32, 4, 2048, 128
REP = HQ // HKV
GW = REP * DH
HG = REP // 2
UB = 4
UM = UB * SQ
NRU = B // UB
NUNIT = HKV * NRU
PW = D // UB
QM = 128
NQC = B * SQ // QM
NSLOT = 8
NITEM = HKV * B
NPRE = 7
SKIPS = (6, 14, 22)
KV_PIECES = (128,) + (192,) * 10
KV_QUEUES = (0, 1, 1)
N_ORDERED = 3
W_ROWS = 32
W_QUEUES = (0, 1)
N_INIT = 88
N_INIT_Q0 = 48
SCALE = (DH ** -0.5) * 1.4426950408889634


def _cut(sizes):
    out, o = [], 0
    for n in sizes:
        out.append((o, n))
        o += n
    return out


def _rows(r0, r1, step):
    return [(o, min(step, r1 - o)) for o in range(r0, r1, step)]


def _kernel(x_hbm, k_hbm, v_hbm, wq_hbm, wo_hbm, out_hbm,
            xw_v, wo_v, kbuf, vbuf, q_scr, o_scr, acc_scr, out_v,
            ksem, vsem, wqsem, wosem, osem):

    def start(copies, queues, first=0):
        for t, c in enumerate(copies):
            c.start(priority=queues[(first + t) % len(queues)])

    def kv_copies(i):
        slot = i % NSLOT
        b = i % B
        g = i // B
        return [pltpu.make_async_copy(src.at[b, g, pl.ds(o, n)], buf.at[slot, pl.ds(o, n)], sem.at[slot])
                for src, buf, sem in ((k_hbm, kbuf, ksem), (v_hbm, vbuf, vsem))
                for o, n in _cut(KV_PIECES)]

    def kv_wait(i):
        slot = i % NSLOT
        pltpu.make_async_copy(kbuf.at[slot], kbuf.at[slot], ksem.at[slot]).wait()
        pltpu.make_async_copy(vbuf.at[slot], vbuf.at[slot], vsem.at[slot]).wait()

    def out_start(r0, r1, sem):
        start([pltpu.make_async_copy(out_v.at[pl.ds(o, n)], out_hbm.at[pl.ds(o, n)], sem)
               for o, n in _rows(r0, r1, W_ROWS)], W_QUEUES)

    def out_wait(r0, r1, sem):
        pltpu.make_async_copy(out_v.at[pl.ds(r0, r1 - r0)], out_v.at[pl.ds(r0, r1 - r0)], sem).wait()

    def o_proj(u, par, c0, ncol):
        g = u // NRU
        ju = u % NRU
        part = jnp.dot(o_scr[par], wo_v[g, :, pl.ds(c0, ncol)], preferred_element_type=jnp.float32)
        tot = acc_scr[ju, :, pl.ds(c0, ncol)] + part
        acc_scr[ju, :, pl.ds(c0, ncol)] = tot
        out_v[pl.ds(pl.multiple_of(ju * UM, UM), UM), pl.ds(c0, ncol)] = tot.astype(jnp.bfloat16)

    def prefetch(i):
        n = i + NPRE
        go = i != SKIPS[0]
        for s in SKIPS:
            n = n - (i >= s).astype(jnp.int32)
            go = jnp.logical_and(go, i != s)

        @pl.when(jnp.logical_and(go, n < NITEM - N_ORDERED))
        def _():
            start(kv_copies(n), KV_QUEUES)

        @pl.when(jnp.logical_and(go, jnp.logical_and(n >= NITEM - N_ORDERED, n < NITEM)))
        def _():
            start(kv_copies(n), (1,))

    def attend(i, oslices):
        g = i // B
        u = i // UB
        par = u % 2
        pos = i % UB
        slot = i % NSLOT
        rq = pl.multiple_of((i % B) * SQ, SQ)
        ro = pl.multiple_of(pos * SQ, SQ)
        k = kbuf[slot]
        v = vbuf[slot]
        scores = []
        for h in range(2):
            qh = jnp.concatenate([q_scr[g, pl.ds(rq, SQ), r * DH:(r + 1) * DH]
                                  for r in range(h * HG, (h + 1) * HG)], axis=0)
            scores.append(lax.dot_general(qh, k, (((1,), (1,)), ((), ())),
                                          preferred_element_type=jnp.float32))
            if h == 0 and oslices:
                ncol = oslices * PW
                o_proj(jnp.maximum(u - 1, 0), 1 - par, pl.multiple_of(pos * ncol, ncol), ncol)
        for h in range(2):
            s = scores[h]
            m = jnp.max(s, axis=1, keepdims=True)
            p = jnp.exp2(s - m)
            l = jnp.sum(p, axis=1, keepdims=True)
            o = jnp.dot(p.astype(jnp.bfloat16), v, preferred_element_type=jnp.float32)
            o = (o / l).astype(jnp.bfloat16)
            for r in range(HG):
                c = (h * HG + r) * DH
                o_scr[par, pl.ds(ro, SQ), c:c + DH] = o[r * SQ:(r + 1) * SQ, :]

    copies = [pltpu.make_async_copy(x_hbm.at[pl.ds(o, n)], xw_v.at[pl.ds(o, n)], wqsem.at[0])
              for o, n in _rows(0, B * SQ, W_ROWS)]
    for g in range(HKV):
        copies += [pltpu.make_async_copy(wq_hbm.at[pl.ds(o, n), pl.ds(g * GW, GW)],
                                         xw_v.at[pl.ds(B * SQ + g * D + o, n)], wqsem.at[g])
                   for o, n in _rows(0, D, W_ROWS)]
    for g in range(HKV):
        copies += [pltpu.make_async_copy(wo_hbm.at[pl.ds(g * GW + o, n)],
                                         wo_v.at[g, pl.ds(o, n)], wosem.at[0])
                   for o, n in _rows(0, GW, W_ROWS)]
    for i in range(NPRE):
        copies += kv_copies(i)
    nchunk = HKV * NQC
    per = -(-(len(copies) - N_INIT) // (nchunk - 1))

    start(copies[:N_INIT_Q0], (0,))
    start(copies[N_INIT_Q0:N_INIT], W_QUEUES, N_INIT_Q0)
    o_scr[1] = jnp.zeros(o_scr.shape[1:], o_scr.dtype)
    acc_scr[...] = jnp.zeros(acc_scr.shape, acc_scr.dtype)

    def q_chunk(c, _):
        def batches(lo, hi):
            first = N_INIT + lo * per
            if first >= len(copies):
                return
            if hi - lo == 1:
                start(copies[first:first + per], W_QUEUES, first)
                return
            mid = (lo + hi) // 2
            pl.when(c - 1 < mid)(lambda: batches(lo, mid))
            pl.when(c - 1 >= mid)(lambda: batches(mid, hi))

        pl.when(c > 0)(lambda: batches(0, nchunk - 1))
        g = c // NQC
        j = c % NQC

        w0 = pl.multiple_of(B * SQ + g * D, B * SQ)

        @pl.when(c == 0)
        def _():
            both = xw_v.at[pl.ds(0, B * SQ + D)]
            pltpu.make_async_copy(both, both, wqsem.at[0]).wait()

        @pl.when(jnp.logical_and(j == 0, c > 0))
        def _():
            slab = xw_v.at[pl.ds(w0, D)]
            pltpu.make_async_copy(slab, slab, wqsem.at[g]).wait()

        r0 = pl.multiple_of(j * QM, QM)
        q = jnp.dot(xw_v[pl.ds(r0, QM), :], xw_v[pl.ds(w0, D), :], preferred_element_type=jnp.float32)
        q_scr[g, pl.ds(r0, QM), :] = (q * SCALE).astype(jnp.bfloat16)
        return 0

    lax.fori_loop(0, nchunk, q_chunk, 0)
    pltpu.make_async_copy(wo_v, wo_v, wosem.at[0]).wait()

    def step(i, _):
        prefetch(i)
        kv_wait(i)
        attend(i, 1)
        return 0

    lax.fori_loop(0, NITEM - UB, step, 0)

    def step_wide(i, _):
        kv_wait(i)
        attend(i, 2)
        return 0

    lax.fori_loop(NITEM - UB, NITEM - 2, step_wide, 0)
    kv_wait(NITEM - 2)
    attend(jnp.int32(NITEM - 2), 0)
    kv_wait(NITEM - 1)
    done = (NRU - 1) * UM
    out_start(0, done, osem.at[0])
    attend(jnp.int32(NITEM - 1), 0)
    half = D // 2
    for t in range(2):
        o_proj(NUNIT - 1, (NUNIT - 1) % 2, t * half, half)
        pltpu.make_async_copy(out_v.at[pl.ds(done, UM), pl.ds(t * half, half)],
                              out_hbm.at[pl.ds(done, UM), pl.ds(t * half, half)],
                              osem.at[1]).start(priority=t)
    out_wait(0, done, osem.at[0])
    out_wait(done, B * SQ, osem.at[1])


@jax.jit
def pallas_standalone__gqa_block_cached__sampling_kernel(
    x: jax.Array,
    k_cache: jax.Array,
    v_cache: jax.Array,
    wq: jax.Array,
    wo: jax.Array,
):
    bf = jnp.bfloat16
    hbm = pl.BlockSpec(memory_space=pl.ANY)
    out = pl.pallas_call(
        _kernel,
        in_specs=[hbm] * 5,
        out_specs=hbm,
        out_shape=jax.ShapeDtypeStruct((B * SQ, D), bf),
        scratch_shapes=[
            pltpu.VMEM((B * SQ + HKV * D, GW), bf),
            pltpu.VMEM((HKV, GW, D), bf),
            pltpu.VMEM((NSLOT, SK, DH), bf),
            pltpu.VMEM((NSLOT, SK, DH), bf),
            pltpu.VMEM((HKV, B * SQ, GW), bf),
            pltpu.VMEM((2, UM, GW), bf),
            pltpu.VMEM((NRU, UM, D), jnp.float32),
            pltpu.VMEM((B * SQ, D), bf),
            pltpu.SemaphoreType.DMA((NSLOT,)),
            pltpu.SemaphoreType.DMA((NSLOT,)),
            pltpu.SemaphoreType.DMA((HKV,)),
            pltpu.SemaphoreType.DMA((1,)),
            pltpu.SemaphoreType.DMA((2,)),
        ],
        compiler_params=pltpu.CompilerParams(
            vmem_limit_bytes=64 * 2**20,
            disable_bounds_checks=True,
            disable_semaphore_checks=True,
        ),
    )(x.reshape(B * SQ, D), k_cache, v_cache, wq, wo)
    return out.reshape(B, SQ, D)
```
